```python
import os as _os
_os.environ.setdefault('JAX_PLATFORMS', 'cpu')
import jax
import jax.numpy as jnp

def _softmax(x, axis=-1):
    return jax.nn.softmax(x, axis=axis)

def _gelu(x):
    return jax.nn.gelu(x, approximate=True)

def _silu(x):
    return jax.nn.silu(x)

def _sigmoid(x):
    return jax.nn.sigmoid(x)

def _layernorm(x, axis=-1, eps=1e-05):
    m = jnp.mean(x, axis=axis, keepdims=True)
    v = jnp.var(x, axis=axis, keepdims=True)
    return (x - m) / jnp.sqrt(v + eps)

def _scatter_add(tgt, idx, src, axis=0):
    return tgt.at[idx].add(src)

def _segment_sum(src, seg, n):
    return jax.ops.segment_sum(src, seg, n)

class _Rng:

    def __init__(self, key):
        self._k = key

    def _next(self):
        self._k, sub = jax.random.split(self._k)
        return sub

    def normal(self, shape):
        return jax.random.normal(self._next(), shape, dtype=jnp.bfloat16)

    def randint(self, lo, hi, shape):
        return jax.random.randint(self._next(), shape, lo, hi, dtype=jnp.int32)

    def uniform(self, shape, lo=0.0, hi=1.0):
        return jax.random.uniform(self._next(), shape, jnp.bfloat16, lo, hi)

    def permutation(self, n):
        return jax.random.permutation(self._next(), n)
kernel_name = 'adaLN_cond__memory_aug_recurrent_mem_tr__moe_arch_mod__prompt'

def setup_inputs():
    _rng = _Rng(jax.random.key(int.from_bytes(__import__("os").urandom(4), "little")))
    _w = lambda a: (lambda t: t.astype(jnp.bfloat16) if jnp.issubdtype(t.dtype, jnp.floating) else t)(jnp.asarray(a))

    def _A_setup():
        B, S, Dm = (1, 2048, 448)
        H, Dh = (16, 256)
        M, seg = (8, 32)
        seg = min(seg, S)
        S = S // seg * seg
        return {'x': _w((lambda *s: _rng.normal(s) * 0.05)(B, S, Dm)), 'mem0': _w((lambda *s: _rng.normal(s) * 0.4)(B, M, Dm)), 'Wq': _w((lambda *s: _rng.normal(s) * 1.6)(Dm, H, Dh) * Dm ** (-0.5)), 'Wk': _w((lambda *s: _rng.normal(s) * 1.6)(Dm, H, Dh) * Dm ** (-0.5)), 'Wv': _w((lambda *s: _rng.normal(s) * 0.4)(Dm, H, Dh) * Dm ** (-0.5)), 'Wo': _w((lambda *s: _rng.normal(s) * 0.4)(H, Dh, Dm) * (H * Dh) ** (-0.5)), 'seg_len': seg}
    _A_in = _A_setup()

    def _B_setup():
        B, S, D, F, C = (1, 2048, 448, 1792, 1)
        return {'x': _w((lambda *s: _rng.normal(s) * 0.05)(B, S, D)), 'w_r': _w((lambda *s: _rng.normal(s) * 0.05)(D)), 'w_gate': _w((lambda *s: _rng.normal(s) * 0.05)(D, F)), 'w_up': _w((lambda *s: _rng.normal(s) * 0.05)(D, F)), 'w_down': _w((lambda *s: _rng.normal(s) * 0.05)(F, D))}
    _B_in = _B_setup()
    return {'A_x': _A_in['x'], 'A_mem0': _A_in['mem0'], 'A_Wq': _A_in['Wq'], 'A_Wk': _A_in['Wk'], 'A_Wv': _A_in['Wv'], 'A_Wo': _A_in['Wo'], 'A_seg_len': _A_in['seg_len'], 'B_x': _B_in['x'], 'B_w_r': _B_in['w_r'], 'B_w_gate': _B_in['w_gate'], 'B_w_up': _B_in['w_up'], 'B_w_down': _B_in['w_down'], 'c': _w((lambda *s: _rng.normal(s) * 0.05)(1, 448) * 8.0), 'w_mod': _w((lambda *s: _rng.normal(s) * 0.05)(448, 6 * 448) * 448 ** (-0.5) * 8.0)}

def reference(A_x, A_mem0, A_Wq, A_Wk, A_Wv, A_Wo, A_seg_len, B_x, B_w_r, B_w_gate, B_w_up, B_w_down, c, w_mod):

    def _A_ref(x, mem0, Wq, Wk, Wv, Wo, seg_len):
        B, S, Dm = x.shape
        H, Dh = (Wq.shape[1], Wq.shape[2])
        M = mem0.shape[1]
        scale = Dh ** (-0.5)
        n_seg = S // seg_len
        L = M + seg_len
        idx = jnp.arange(L)
        mask = (idx[:, None] < M) | (idx[:, None] >= idx[None, :])
        mem = mem0
        outs = []
        for s in range(n_seg):
            xs = x[:, s * seg_len:(s + 1) * seg_len, :].copy()
            h = jnp.concatenate([mem, xs], axis=1)
            q = jnp.einsum('btd,dhe->bhte', h, Wq)
            k = jnp.einsum('btd,dhe->bhte', h, Wk)
            v = jnp.einsum('btd,dhe->bhte', h, Wv)
            scores = jnp.einsum('bhqe,bhke->bhqk', q, k) * scale
            scores = jnp.where(mask[None, None], scores, -1000000000.0)
            p = _softmax(scores, axis=-1)
            o = jnp.einsum('bhqk,bhke->bhqe', p, v)
            o = jnp.einsum('bhte,hed->btd', o, Wo)
            mem = o[:, :M, :].copy()
            outs.append(o[:, M:, :])
        return jnp.concatenate(outs, axis=1)

    def _B_ref(x, w_r, w_gate, w_up, w_down):
        B, S, D = x.shape
        C = 1
        r = x @ w_r
        idx = jnp.argsort(-r, axis=-1)[:, :C]
        idx_e = jnp.repeat(idx.reshape(B, C, 1), D, axis=2)
        x_sel = jnp.take_along_axis(x, idx_e, axis=1)
        g = _silu(x_sel @ w_gate)
        u = x_sel @ w_up
        y = g * u @ w_down
        r_sel = _sigmoid(jnp.take_along_axis(r, idx, axis=1))
        y = y * r_sel.reshape(B, C, 1)
        b_off = (jnp.arange(B) * S).reshape(B, 1)
        flat_idx = (idx + b_off).reshape(B * C)
        zero = (x * 0.0).reshape(B * S, D)
        upd = _scatter_add(zero, flat_idx, y.reshape(B * C, D), axis=0)
        return x + upd.reshape(B, S, D)
    x = A_x
    mod = (_silu(c) @ w_mod).reshape(c.shape[0], 6, 1, -1)
    sa, ca, ga, sb, cb, gb = (mod[:, 0].copy(), mod[:, 1].copy(), mod[:, 2].copy(), mod[:, 3].copy(), mod[:, 4].copy(), mod[:, 5].copy())
    h = _layernorm(x, axis=-1) * (1 + ca) + sa
    x = x + ga * _A_ref(h, A_mem0, A_Wq, A_Wk, A_Wv, A_Wo, A_seg_len)
    h = _layernorm(x, axis=-1) * (1 + cb) + sb
    x = x + gb * _B_ref(h, B_w_r, B_w_gate, B_w_up, B_w_down)
    return x
```

```python
import functools

import jax
import jax.numpy as jnp
import jax.experimental.pallas as pl
import jax.experimental.pallas.tpu as pltpu

F32 = jnp.float32
BF16 = jnp.bfloat16
U32 = jnp.uint32

S = 2048
D = 448
DP = 512
H = 16
DH = 256
NM = 8
SEG = 32
FF = 1792
NPAIR = H // 2
NT = 7
TB = 128
NBLK = S // TB
EPS = 1e-5
CH = 64
NCH = D // CH
TDIMS = (((1,), (1,)), ((), ()))


def _pack2(lo, hi):
    return pltpu.bitcast(pltpu.pack_elementwise([lo, hi], packed_dtype=BF16), U32)


def _key_allreduce(v, op, lane):
    for k in (2, 4, 8):
        up = pltpu.roll(v, k, 1)
        dn = pltpu.roll(v, 128 - k, 1)
        v = op(v, jnp.where((lane & k) != 0, up, dn))
    return v


def _fold8(v):
    acc = v[0:8]
    for i in range(1, v.shape[0] // 8):
        acc = acc + v[8 * i:8 * i + 8]
    return acc


def _kernel(xt_hbm, mem0_ref, wq_hbm, wk_hbm, wv_hbm, wot_hbm, wr_ref, wgate_hbm,
            wup_hbm, wdt_hbm, c_ref, wmod_hbm, out_hbm,
            wraw, wot_s, wmod_s, wgate_s, wup_s, wdt_s, xs, wg_s, wu_s, modt, hbuf,
            abuf, gbuf, ubuf, o32, obf, h2s, rbuf, kx, zsm,
            sem_w, sem_x, sem_f, sem_o):
    def half_copies(w_hbm, wi, r0, nrows, s0):
        return [pltpu.make_async_copy(w_hbm.at[pl.ds(r0, nrows), pl.ds(e * 128, 128)],
                                      wraw.at[wi * 2 + e, pl.ds(r0, nrows)],
                                      sem_w.at[s0 + e]) for e in range(2)]
    k_cp = half_copies(wk_hbm, 1, 0, D * H, 0)
    q_cp = [half_copies(wq_hbm, 0, 0, 128 * H, 2),
            half_copies(wq_hbm, 0, 128 * H, 128 * H, 4),
            half_copies(wq_hbm, 0, 256 * H, 192 * H, 6)]
    v_cp = half_copies(wv_hbm, 2, 0, D * H, 8)
    o_cp = [pltpu.make_async_copy(wot_hbm.at[pl.ds(0, 6)], wot_s.at[pl.ds(0, 6)],
                                  sem_w.at[10]),
            pltpu.make_async_copy(wot_hbm.at[pl.ds(6, 10)], wot_s.at[pl.ds(6, 10)],
                                  sem_w.at[11])]
    mod_cp = pltpu.make_async_copy(wmod_hbm, wmod_s, sem_w.at[12])
    x_cp = [pltpu.make_async_copy(xt_hbm.at[:, pl.ds(b * TB, TB)], xs.at[b], sem_x.at[b])
            for b in range(NBLK)]
    f_cp = [pltpu.make_async_copy(src, dst, sem_f.at[i]) for i, (src, dst) in
            enumerate(((wgate_hbm, wgate_s), (wup_hbm, wup_s), (wdt_hbm, wdt_s)))]
    for cp in k_cp + q_cp[0] + q_cp[1] + q_cp[2] + v_cp + o_cp + [x_cp[0], mod_cp]:
        cp.start()
    zsm[0] = 0

    def heads(wi, hp, d0=0, nd=D):
        los, his = [], []
        for e in range(2):
            w32 = wraw.at[wi * 2 + e].bitcast(U32)
            v = w32[pl.ds(d0 * 8 + hp, nd, stride=8), :]
            los.append(pltpu.bitcast(v << 16, F32).astype(BF16))
            his.append(pltpu.bitcast(v & jnp.uint32(0xFFFF0000), F32).astype(BF16))
        return jnp.concatenate(los, axis=1), jnp.concatenate(his, axis=1)

    def bf(v):
        return pltpu.bitcast(v, BF16)

    z64 = jnp.zeros((64, DH), BF16)

    def put_tile(w_s, n, tv):
        pk = pltpu.bitcast(tv.astype(BF16), U32)
        w_s[n, 0:D // 2, :] = pk
        w_s[n, D // 2:DP // 2, :] = pk[192:224]

    def tdot(a, b):
        return jax.lax.dot_general(a, b, TDIMS, preferred_element_type=F32)

    def zmask(dep):
        return pltpu.bitcast(dep, jnp.int32) & jnp.full((8, 128), zsm[0], jnp.int32)

    def tie(lhs, dep):
        l32 = pltpu.bitcast(lhs, jnp.int32)
        top = jnp.concatenate([l32[0:8, 0:128] | zmask(dep), l32[0:8, 128:]], axis=1)
        return pltpu.bitcast(jnp.concatenate([top, l32[8:]], axis=0), BF16)

    def gate(v, z):
        if z is None:
            return v
        zz = z[0:1] if v.shape[0] == 1 else jnp.concatenate([z] * (v.shape[0] // 8), axis=0)
        return pltpu.bitcast(pltpu.bitcast(v, jnp.int32) | zz, F32)

    class Side:
        def __init__(self, gen):
            self.gen, self.started, self.z = gen, False, None

        def stage(self):
            if self.gen is None:
                return None
            try:
                if not self.started:
                    self.started = True
                    next(self.gen)
                return self.gen.send(self.z)
            except StopIteration:
                self.gen = None
                return None

        def after(self, res):
            self.z = zmask(res) if self.gen is not None else None

    scale = float(DH) ** -0.5
    for cp in k_cp:
        cp.wait()
    for j in range(4):
        if j < 3:
            for cp in q_cp[j]:
                cp.wait()
        for p in range(NPAIR):
            if j == 0:
                k_e, k_o = heads(1, p)
                kx[2 * p] = pltpu.bitcast(k_e, U32)
                kx[2 * p + 1] = pltpu.bitcast(k_o, U32)
            else:
                k_e, k_o = bf(kx[2 * p]), bf(kx[2 * p + 1])
            if j < 3:
                q_e, q_o = heads(0, p, j * 128, 128)
                put_tile(wg_s, p * NT + j, tdot(k_e, q_e) * scale)
                put_tile(wg_s, p * NT + 4 + j, tdot(k_o, q_o) * scale)
            else:
                q_e, q_o = heads(0, p, 384, 64)
                t3 = (tdot(k_e, jnp.concatenate([q_e, z64], axis=0))
                      + tdot(k_o, jnp.concatenate([z64, q_o], axis=0)))
                put_tile(wg_s, p * NT + 3, t3 * scale)

    def fuse_vo(p, side=None):
        v_e, v_o = heads(2, p)
        r_e, r_o = wot_s[2 * p], wot_s[2 * p + 1]
        for t in range(NT):
            dep = side.stage() if side is not None else None
            if t < 3:
                tv = tdot(v_e, r_e[t * 128:(t + 1) * 128])
            elif t == 3:
                tv = (tdot(v_e, jnp.concatenate([r_e[384:], z64], axis=0))
                      + tdot(v_o, jnp.concatenate([z64, r_o[384:]], axis=0)))
            else:
                tv = tdot(v_o, r_o[(t - 4) * 128:(t - 3) * 128])
            put_tile(wu_s, p * NT + t, tv)
            if side is not None:
                side.after(tv[0:8])
            if dep is not None:
                v_e, v_o = tie(v_e, dep), tie(v_o, dep)

    for cp in v_cp:
        cp.wait()
    o_cp[0].wait()
    for p in range(3):
        fuse_vo(p)
    o_cp[1].wait()
    for p in range(3, NPAIR - 2):
        fuse_vo(p)

    x_cp[0].wait()
    mod_cp.wait()
    for cp in x_cp[1:] + f_cp:
        cp.start()
    cvec = c_ref[...].astype(F32)
    sc = cvec * jax.nn.sigmoid(cvec)
    sc = jnp.broadcast_to(sc, (16, D)).astype(BF16)
    mod = jnp.dot(sc, wmod_s[...], preferred_element_type=F32)[0:1]
    mod = mod.astype(BF16).astype(F32)
    col = jax.lax.broadcasted_iota(jnp.int32, (1, 6 * D), 1)
    is_scale = ((col >= D) & (col < 2 * D)) | ((col >= 4 * D) & (col < 5 * D))
    mod = jnp.where(is_scale, 1.0 + mod, mod)
    wr = wr_ref[...].astype(F32).reshape(1, D)
    row = jnp.concatenate([mod, wr, jnp.zeros((1, 64), F32)], axis=1)
    for i in range(25):
        blk = jnp.broadcast_to(row[:, i * 128:(i + 1) * 128], (128, 128))
        modt[i * 128:(i + 1) * 128, :] = blk.T

    def mcol(i, r0, n):
        return modt[i * D + r0:i * D + r0 + n, :]

    TILES = ((0, 128), (128, 128), (256, 128), (384, 64))

    def var_stages(src, mu, z):
        acc = None
        for r0, n in TILES:
            xc = src(r0, n) - gate(mu, z)
            f = _fold8(xc * xc)
            acc = f if acc is None else acc + f
            z = yield acc
        var = jnp.sum(acc, axis=0, keepdims=True) * (1.0 / D)
        return jax.lax.rsqrt(var + EPS), z

    def ln1_stages(b):
        src = lambda r0, n: xs[b, r0:r0 + n, :].astype(F32)
        z = yield
        acc = None
        for r0, n in TILES:
            f = _fold8(gate(src(r0, n), z))
            acc = f if acc is None else acc + f
            z = yield acc
        mu = jnp.sum(acc, axis=0, keepdims=True) * (1.0 / D)
        rstd, z = yield from var_stages(src, mu, z)
        for t, (r0, n) in enumerate(TILES):
            ht = (src(r0, n) - gate(mu, z)) * rstd * mcol(1, r0, n) + mcol(0, r0, n)
            if n == 64:
                ht = jnp.concatenate([ht, ht], axis=0)
            tile = ht.T
            hbuf[b, :, t * 128:(t + 1) * 128] = tile
            z = yield tile[120:128]

    def out_stages(b):
        z = yield
        acc = None
        for t, (r0, n) in enumerate(TILES):
            a = gate(abuf[:, t * 128:(t + 1) * 128], z).T
            if n == 64:
                a = a[:64] + a[64:]
            x1 = xs[b, r0:r0 + n, :].astype(F32) + mcol(2, r0, n) * a
            o32[b, r0:r0 + n, :] = x1
            f = _fold8(x1)
            acc = f if acc is None else acc + f
            z = yield acc
        mu = jnp.sum(acc, axis=0, keepdims=True) * (1.0 / D)
        src = lambda r0, n: o32[b, r0:r0 + n, :]
        rstd, z = yield from var_stages(src, mu, z)
        racc = None
        for ch in range(NCH):
            r0 = ch * CH
            x1 = src(r0, CH)
            h2 = (x1 - gate(mu, z)) * rstd * mcol(4, r0, CH) + mcol(3, r0, CH)
            o = x1 + mcol(5, r0, CH) * h2
            o32[b, r0:r0 + CH, :] = o
            obf[b, r0:r0 + CH, :] = o.astype(BF16)
            h2s[b, r0:r0 + CH, :] = h2.astype(BF16)
            f = _fold8(h2 * mcol(6, r0, CH))
            racc = f if racc is None else racc + f
            if ch == NCH - 1:
                rbuf[pl.ds(b, 1), :] = jnp.sum(racc, axis=0, keepdims=True)
            z = yield racc + o[CH - 8:]

    side = Side(ln1_stages(0))
    fuse_vo(NPAIR - 2, side)
    fuse_vo(NPAIR - 1, side)

    lane8 = jax.lax.broadcasted_iota(jnp.int32, (8, 128), 1)
    lo_half = lane8 < 64
    lane40 = jax.lax.broadcasted_iota(jnp.int32, (40, 128), 1)
    row40 = jax.lax.broadcasted_iota(jnp.int32, (40, 128), 0)

    def proj_pair(lhs, w_s, buf, p, dests):
        r = [jnp.dot(lhs, bf(w_s[p * NT + t]), preferred_element_type=F32)
             for t in range(NT)]
        for g, (slot, jhi) in enumerate(dests):
            rows = slice(8 * g, 8 * g + 8)
            base = jhi * 64 + p * 8
            for t in range(3):
                buf[slot, t, base:base + 8, :] = _pack2(r[t][rows], r[4 + t][rows])
            t3 = r[3][rows]
            buf[slot, 3, base:base + 8, :] = _pack2(jnp.where(lo_half, t3, 0.0),
                                                    jnp.where(lo_half, 0.0, t3))
        return r[0][0:8]

    def xgroup(v):
        return jnp.concatenate([v[:, :384], jnp.where(lo_half, v[:, 384:], 0.0)], axis=1)

    def step(groups, dests, xq, mem, slot, side=None):
        lhs = jnp.concatenate(groups, axis=0).astype(BF16)

        def proj(lhs, w_s, buf, p):
            dep = side.stage() if side is not None else None
            res = proj_pair(lhs, w_s, buf, p, dests)
            if side is not None:
                side.after(res)
            return lhs if dep is None else tie(lhs, dep)

        for p in range(NPAIR):
            lhs = proj(lhs, wg_s, gbuf, p)
        lhs = proj(lhs, wu_s, ubuf, 0)
        m3 = mem[:, 384:]
        memq = jnp.concatenate([mem[:, :384], m3 + pltpu.roll(m3, 64, 1)], axis=1)
        q = jnp.concatenate([xq, memq], axis=0).astype(BF16)
        gmat = jnp.concatenate([bf(gbuf[slot, t]) for t in range(4)], axis=1)
        s = tdot(q, gmat)
        sj = []
        for jhi in range(5):
            blk = s[:, jhi * 128:(jhi + 1) * 128]
            if jhi < 4:
                key = jhi * 8 + ((lane40 >> 1) & 7)
                blk = jnp.where(row40 >= key, blk, -1000000000.0)
            sj.append(blk)
        m = functools.reduce(jnp.maximum, sj)
        m = _key_allreduce(m, jnp.maximum, lane40)
        ej = [jnp.exp(b - m) for b in sj]
        den = functools.reduce(jnp.add, ej)
        den = _key_allreduce(den, jnp.add, lane40)
        inv = 1.0 / den
        pmat = jnp.concatenate([e * inv for e in ej], axis=1).astype(BF16)
        for p in range(1, NPAIR):
            lhs = proj(lhs, wu_s, ubuf, p)
        umat = jnp.concatenate([bf(ubuf[slot, t]) for t in range(4)], axis=1)
        return jnp.dot(pmat, umat, preferred_element_type=F32)

    def out_copy(b):
        return pltpu.make_async_copy(obf.at[b], out_hbm.at[:, pl.ds(b * TB, TB)], sem_o.at[b])

    abuf[...] = jnp.zeros((TB, DP), F32)

    def blk_body(t, mem):
        @pl.when(t >= 2)
        def _():
            b = t - 2
            pltpu.make_async_copy(
                obf.at[b], out_hbm.at[:, pl.ds(pl.multiple_of(b * TB, TB), TB)],
                sem_o.at[b]).start()

        @pl.when(t < NBLK - 1)
        def _():
            b = t + 1
            pltpu.make_async_copy(
                xt_hbm.at[:, pl.ds(pl.multiple_of(b * TB, TB), TB)], xs.at[b],
                sem_x.at[b]).wait()

        for half in range(2):
            r0 = half * 64
            xa = hbuf[t, r0:r0 + SEG, :]
            xb = hbuf[t, r0 + SEG:r0 + 2 * SEG, :]
            ga_ = [xgroup(xa[8 * g:8 * g + 8]) for g in range(4)]
            gb_ = [xgroup(xb[8 * g:8 * g + 8]) for g in range(4)]
            side = Side(out_stages(jnp.maximum(t - 1, 0)) if half == 0
                        else ln1_stages(jnp.minimum(t + 1, NBLK - 1)))
            o = step(ga_ + [mem, gb_[3]],
                     [(0, 0), (0, 1), (0, 2), (0, 3), (0, 4), (1, 3)], xa, mem, 0, side)
            mem = o[32:40]
            abuf[r0:r0 + SEG, :] = o[0:32]
            o = step(gb_[:3] + [mem], [(1, 0), (1, 1), (1, 2), (1, 4)], xb, mem, 1)
            mem = o[32:40]
            abuf[r0 + SEG:r0 + 2 * SEG, :] = o[0:32]
        return mem

    m0 = mem0_ref[...].astype(F32)
    mem0 = jnp.concatenate([m0, jnp.zeros((NM, 64), F32)], axis=1)
    jax.lax.fori_loop(0, NBLK, blk_body, mem0)
    out_copy(NBLK - 2).start()
    for _ in out_stages(NBLK - 1):
        pass
    out_copy(NBLK - 1).start()

    for cp in f_cp:
        cp.wait()
    rb = rbuf[...]
    rmax = jnp.max(jnp.max(rb, axis=0, keepdims=True), axis=1, keepdims=True)
    tok = (jax.lax.broadcasted_iota(jnp.int32, (NBLK, TB), 0) * TB
           + jax.lax.broadcasted_iota(jnp.int32, (NBLK, TB), 1))
    idx = jnp.min(jnp.where(rb == rmax, tok, S - 1))
    bsel = idx // TB
    lsel = idx - bsel * TB
    onehot = (jax.lax.broadcasted_iota(jnp.int32, (16, TB), 1) == lsel)
    onehot = jnp.where(onehot, 1.0, 0.0).astype(BF16)
    hsel = tdot(onehot, h2s[bsel]).astype(BF16)
    gate = jnp.dot(hsel, wgate_s[...], preferred_element_type=F32)
    up = jnp.dot(hsel, wup_s[...], preferred_element_type=F32)
    act = (gate * jax.nn.sigmoid(gate) * up)[0:1]
    rsel = jax.lax.broadcasted_iota(jnp.int32, (TB, FF), 0) == lsel
    actm = jnp.where(rsel, jnp.broadcast_to(act, (TB, FF)), 0.0).astype(BF16)
    yt = tdot(wdt_s[...], actm)
    yt = yt * jax.nn.sigmoid(rmax)
    for b in range(NBLK):
        out_copy(b).wait()
    obf[bsel] = (o32[bsel] + modt[5 * D:6 * D, :] * yt).astype(BF16)
    fix = pltpu.make_async_copy(
        obf.at[bsel], out_hbm.at[:, pl.ds(pl.multiple_of(bsel * TB, TB), TB)], sem_o.at[0])
    fix.start()
    fix.wait()


@jax.jit
def _run(A_x, A_mem0, A_Wq, A_Wk, A_Wv, A_Wo, B_w_r, B_w_gate, B_w_up, B_w_down, c, w_mod):
    xt = jnp.transpose(A_x.reshape(S, D))
    mem0 = A_mem0.reshape(NM, D)
    wq = A_Wq.reshape(D * H, DH)
    wk = A_Wk.reshape(D * H, DH)
    wv = A_Wv.reshape(D * H, DH)
    wot = jnp.transpose(A_Wo, (0, 2, 1))
    wdt = jnp.transpose(B_w_down)
    vmem = pl.BlockSpec(memory_space=pltpu.VMEM)
    hbm = pl.BlockSpec(memory_space=pl.ANY)
    out_t = pl.pallas_call(
        _kernel,
        out_shape=jax.ShapeDtypeStruct((D, S), BF16),
        in_specs=[hbm, vmem, hbm, hbm, hbm, hbm, vmem, hbm, hbm, hbm, vmem, hbm],
        out_specs=hbm,
        scratch_shapes=[
            pltpu.VMEM((6, D * H, 128), BF16),
            pltpu.VMEM((H, D, DH), BF16),
            pltpu.VMEM((D, 6 * D), BF16),
            pltpu.VMEM((D, FF), BF16),
            pltpu.VMEM((D, FF), BF16),
            pltpu.VMEM((D, FF), BF16),
            pltpu.VMEM((NBLK, D, TB), BF16),
            pltpu.VMEM((NPAIR * NT, DP // 2, 128), U32),
            pltpu.VMEM((NPAIR * NT, DP // 2, 128), U32),
            pltpu.VMEM((25 * 128, 128), F32),
            pltpu.VMEM((NBLK, TB, DP), F32),
            pltpu.VMEM((TB, DP), F32),
            pltpu.VMEM((2, 4, 320, 128), U32),
            pltpu.VMEM((2, 4, 320, 128), U32),
            pltpu.VMEM((NBLK, D, TB), F32),
            pltpu.VMEM((NBLK, D, TB), BF16),
            pltpu.VMEM((NBLK, D, TB), BF16),
            pltpu.VMEM((NBLK, TB), F32),
            pltpu.VMEM((H, D // 2, DH), U32),
            pltpu.SMEM((1,), jnp.int32),
            pltpu.SemaphoreType.DMA((13,)),
            pltpu.SemaphoreType.DMA((NBLK,)),
            pltpu.SemaphoreType.DMA((3,)),
            pltpu.SemaphoreType.DMA((NBLK,)),
        ],
        compiler_params=pltpu.CompilerParams(vmem_limit_bytes=110 * 1024 * 1024),
    )(xt, mem0, wq, wk, wv, wot, B_w_r, B_w_gate, B_w_up, wdt, c, w_mod)
    return jnp.transpose(out_t).reshape(1, S, D)


def pallas_adaLN_cond__memory_aug_recurrent_mem_tr__moe_arch_mod__prompt_kernel(
    A_x, A_mem0, A_Wq, A_Wk, A_Wv, A_Wo, A_seg_len, B_x, B_w_r, B_w_gate, B_w_up,
    B_w_down, c, w_mod,
):
    del A_seg_len, B_x
    return _run(A_x, A_mem0, A_Wq, A_Wk, A_Wv, A_Wo, B_w_r, B_w_gate, B_w_up, B_w_down,
                c, w_mod)
```

```python
import functools

import jax
import jax.numpy as jnp
import jax.experimental.pallas as pl
import jax.experimental.pallas.tpu as pltpu

F32 = jnp.float32
BF16 = jnp.bfloat16
U32 = jnp.uint32

S = 2048
D = 448
DM = 384
DP = 512
H = 16
DH = 256
NM = 8
SEG = 32
FF = 1792
NPAIR = H // 2
NT = 7
TB = 128
NBLK = S // TB
EPS = 1e-5
CH = 64
NCH = D // CH
TDIMS = (((1,), (1,)), ((), ()))


def _pack2(lo, hi):
    return pltpu.bitcast(pltpu.pack_elementwise([lo, hi], packed_dtype=BF16), U32)


def _key_allreduce(v, op, lane):
    for k in (2, 4, 8):
        up = pltpu.roll(v, k, 1)
        dn = pltpu.roll(v, 128 - k, 1)
        v = op(v, jnp.where((lane & k) != 0, up, dn))
    return v


def _fold8(v):
    acc = v[0:8]
    for i in range(1, v.shape[0] // 8):
        acc = acc + v[8 * i:8 * i + 8]
    return acc


def _kernel(xt_hbm, mem0_ref, wq_hbm, wk_hbm, wv_hbm, wot_hbm, wr_ref, wgate_hbm,
            wup_hbm, wdt_hbm, c_ref, wmod_hbm, out_hbm,
            wraw, wot_s, wmod_s, wgate_s, wup_s, wdt_s, xs, wg_s, wu_s, modt, hbuf,
            abuf, gbuf, ubuf, o32, obf, h2s, rbuf, hx, wy_s, wb_s, ybuf, zsm,
            sem_w, sem_x, sem_f, sem_o):
    def half_copies(w_hbm, wi, r0, nrows, s0):
        return [pltpu.make_async_copy(w_hbm.at[pl.ds(r0, nrows), pl.ds(e * 128, 128)],
                                      wraw.at[wi * 2 + e, pl.ds(r0, nrows)],
                                      sem_w.at[s0 + e]) for e in range(2)]
    KH = D // 2
    k_cp = [half_copies(wk_hbm, 1, 0, KH * H, 0), half_copies(wk_hbm, 1, KH * H, KH * H, 2)]
    q_cp = [half_copies(wq_hbm, 0, 0, 128 * H, 4),
            half_copies(wq_hbm, 0, 128 * H, 128 * H, 6),
            half_copies(wq_hbm, 0, 256 * H, 192 * H, 8)]
    v_cp = half_copies(wv_hbm, 2, 0, D * H, 10)
    o_cp = [pltpu.make_async_copy(wot_hbm.at[pl.ds(h0, nh)], wot_s.at[pl.ds(h0, nh)],
                                  sem_w.at[12 + i])
            for i, (h0, nh) in enumerate(((0, 4), (4, 6), (10, 6)))]
    mod_cp = pltpu.make_async_copy(wmod_hbm, wmod_s, sem_w.at[15])
    x_cp = [pltpu.make_async_copy(xt_hbm.at[:, pl.ds(b * TB, TB)], xs.at[b], sem_x.at[b])
            for b in range(NBLK)]
    f_cp = [pltpu.make_async_copy(src, dst, sem_f.at[i]) for i, (src, dst) in
            enumerate(((wgate_hbm, wgate_s), (wup_hbm, wup_s), (wdt_hbm, wdt_s)))]
    for cp in (k_cp[0] + q_cp[0] + k_cp[1] + q_cp[1] + q_cp[2] + v_cp + o_cp
               + [x_cp[0], mod_cp]):
        cp.start()
    zsm[0] = 0

    def bf(v):
        return pltpu.bitcast(v, BF16)

    def ldw(ref, n, r0=0, r1=None):
        r1 = ref.shape[1] if r1 is None else r1
        return bf(ref.bitcast(U32)[n, r0 // 2:r1 // 2, :])

    def heads(wi, hp, d0=0, nd=D, mul=None):
        for e in range(2):
            w32 = wraw.at[wi * 2 + e].bitcast(U32)
            v = w32[pl.ds(d0 * 8 + hp, nd, stride=8), :]
            lo = pltpu.bitcast(v << 16, F32)
            hi = pltpu.bitcast(v & jnp.uint32(0xFFFF0000), F32)
            if mul is not None:
                lo, hi = lo * mul, hi * mul
            hx[(wi * H + 2 * hp) * 2 + e, d0:d0 + nd, :] = lo.astype(BF16)
            hx[(wi * H + 2 * hp + 1) * 2 + e, d0:d0 + nd, :] = hi.astype(BF16)

    def head(wi, h, d0=0, nd=D):
        return jnp.concatenate([ldw(hx, (wi * H + h) * 2 + e, d0, d0 + nd)
                                for e in range(2)], axis=1)

    z64 = jnp.zeros((64, DH), BF16)

    def tdot(a, b):
        return jax.lax.dot_general(a, b, TDIMS, preferred_element_type=F32)

    def zmask(dep):
        return pltpu.bitcast(dep, jnp.int32) & jnp.full((8, 128), zsm[0], jnp.int32)

    def tie(lhs, dep):
        l32 = pltpu.bitcast(lhs, jnp.int32)
        top = jnp.concatenate([l32[0:8, 0:128] | zmask(dep), l32[0:8, 128:]], axis=1)
        return pltpu.bitcast(jnp.concatenate([top, l32[8:]], axis=0), BF16)

    def gate(v, z):
        if z is None:
            return v
        zz = z[0:1] if v.shape[0] == 1 else jnp.concatenate([z] * (v.shape[0] // 8), axis=0)
        return pltpu.bitcast(pltpu.bitcast(v, jnp.int32) | zz, F32)

    class Side:
        def __init__(self, gen):
            self.gen, self.started, self.z, self.budget = gen, False, None, 1000

        def stage(self):
            if self.gen is None or self.budget == 0:
                return None
            self.budget -= 1
            try:
                if not self.started:
                    self.started = True
                    next(self.gen)
                return self.gen.send(self.z)
            except StopIteration:
                self.gen = None
                return None

        def after(self, res):
            self.z = zmask(res) if self.gen is not None else None

    scale = float(DH) ** -0.5

    def a_tiles(p, j, r0, r1):
        a_e = tdot(head(1, 2 * p, r0, r1 - r0), head(0, 2 * p, j * 128, 128))
        a_o = tdot(head(1, 2 * p + 1, r0, r1 - r0), head(0, 2 * p + 1, j * 128, 128))
        rm = min(r1, DM)
        wg_s[p * NT + j, r0:rm, :] = a_e[:rm - r0].astype(BF16)
        wg_s[p * NT + 4 + j, r0:rm, :] = a_o[:rm - r0].astype(BF16)
        if r1 > DM:
            wy = jnp.concatenate([a_e[DM - r0:], a_o[DM - r0:]], axis=0).T
            wy_s[p, j * 128:(j + 1) * 128, :] = wy.astype(BF16)

    def tail_t(l_e, l_o, r_e, r_o):
        t_e = tdot(l_e, jnp.concatenate([r_e, z64], axis=0))
        t_o = tdot(l_o, jnp.concatenate([r_o[:DM], z64, r_o[DM:]], axis=0))
        return t_e, t_o

    for half in range(2):
        for cp in k_cp[half] + (q_cp[0] if half == 0 else []):
            cp.wait()
        for p in range(NPAIR):
            heads(1, p, half * KH, KH)
            if half == 0:
                heads(0, p, 0, 128, scale)
            a_tiles(p, 0, half * KH, (half + 1) * KH)
    for j in (1, 2):
        for cp in q_cp[j]:
            cp.wait()
        for p in range(NPAIR):
            heads(0, p, j * 128, 128, scale)
            a_tiles(p, j, 0, D)
    for p in range(NPAIR):
        heads(0, p, DM, 64, scale)
        t_e, t_o = tail_t(head(0, 2 * p, DM, 64), head(0, 2 * p + 1, DM, 64),
                          head(1, 2 * p), head(1, 2 * p + 1))
        for i in range(3):
            blk = jnp.concatenate([t_e[:, i * 128:(i + 1) * 128],
                                   t_o[:, i * 128:(i + 1) * 128]], axis=0).T
            wg_s[p * NT + 3, i * 128:(i + 1) * 128, :] = blk.astype(BF16)
        wy = (t_e[:, DM:] + t_o[:, DM:]).astype(BF16)
        wy_s[p, DM:D, :] = wy

    def fuse_vo(p, side=None):
        heads(2, p)
        v_e, v_o = head(2, 2 * p), head(2, 2 * p + 1)
        r_e, r_o = wot_s[2 * p], wot_s[2 * p + 1]
        for t in (3, 0, 1, 2, 4, 5, 6):
            dep = side.stage() if side is not None else None
            if t == 3:
                t_e, t_o = tail_t(r_e[DM:], r_o[DM:], v_e, v_o)
                for i in range(4):
                    blk = jnp.concatenate([t_e[:, i * 128:(i + 1) * 128],
                                           t_o[:, i * 128:(i + 1) * 128]], axis=0).T
                    if i < 3:
                        wu_s[p * NT + 3, i * 128:(i + 1) * 128, :] = blk.astype(BF16)
                    else:
                        wb_s[3, p * 128:(p + 1) * 128, :] = blk.astype(BF16)
                res = t_e[0:8, 0:128]
            else:
                tv = (tdot(v_e, r_e[t * 128:(t + 1) * 128]) if t < 3
                      else tdot(v_o, r_o[(t - 4) * 128:(t - 3) * 128]))
                wu_s[p * NT + t] = tv[:DM].astype(BF16)
                r0 = p * 128 + (64 if t > 3 else 0)
                wb_s[t % 4, r0:r0 + 64, :] = tv[DM:].astype(BF16)
                res = tv[0:8]
            if side is not None:
                side.after(res)
            if dep is not None:
                v_e, v_o = tie(v_e, dep), tie(v_o, dep)

    for cp in v_cp:
        cp.wait()
    for i, pairs in enumerate(((0, 1), (2, 3, 4), (5,))):
        o_cp[i].wait()
        for p in pairs:
            fuse_vo(p)

    x_cp[0].wait()
    mod_cp.wait()
    for cp in x_cp[1:] + f_cp:
        cp.start()
    cvec = c_ref[...].astype(F32)
    sc = cvec * jax.nn.sigmoid(cvec)
    sc = jnp.broadcast_to(sc, (16, D)).astype(BF16)
    mod = jnp.dot(sc, wmod_s[...], preferred_element_type=F32)[0:1]
    mod = mod.astype(BF16).astype(F32)
    col = jax.lax.broadcasted_iota(jnp.int32, (1, 6 * D), 1)
    is_scale = ((col >= D) & (col < 2 * D)) | ((col >= 4 * D) & (col < 5 * D))
    mod = jnp.where(is_scale, 1.0 + mod, mod)
    wr = wr_ref[...].astype(F32).reshape(1, D)
    row = jnp.concatenate([mod, wr, jnp.zeros((1, 64), F32)], axis=1)
    for i in range(25):
        blk = jnp.broadcast_to(row[:, i * 128:(i + 1) * 128], (128, 128))
        modt[i * 128:(i + 1) * 128, :] = blk.T

    def mcol(i, r0, n):
        return modt[i * D + r0:i * D + r0 + n, :]

    TILES = ((0, 128), (128, 128), (256, 128), (384, 64))

    def var_stages(src, mu, z):
        acc = None
        for r0, n in TILES:
            xc = src(r0, n) - gate(mu, z)
            f = _fold8(xc * xc)
            acc = f if acc is None else acc + f
            z = yield acc
        var = jnp.sum(acc, axis=0, keepdims=True) * (1.0 / D)
        return jax.lax.rsqrt(var + EPS), z

    def ln1_stages(b):
        src = lambda r0, n: xs[b, r0:r0 + n, :].astype(F32)
        z = yield
        acc = None
        for r0, n in TILES:
            f = _fold8(gate(src(r0, n), z))
            acc = f if acc is None else acc + f
            z = yield acc
        mu = jnp.sum(acc, axis=0, keepdims=True) * (1.0 / D)
        rstd, z = yield from var_stages(src, mu, z)
        for t, (r0, n) in enumerate(TILES):
            ht = (src(r0, n) - gate(mu, z)) * rstd * mcol(1, r0, n) + mcol(0, r0, n)
            if n == 64:
                ht = jnp.concatenate([ht, ht], axis=0)
            tile = ht.T
            hbuf[b, :, t * 128:(t + 1) * 128] = tile
            z = yield tile[120:128]

    def out_stages(b):
        z = yield
        acc = None
        for t, (r0, n) in enumerate(TILES):
            a = gate(abuf[:, t * 128:(t + 1) * 128], z).T
            if n == 64:
                a = a[:64] + a[64:]
            x1 = xs[b, r0:r0 + n, :].astype(F32) + mcol(2, r0, n) * a
            o32[b, r0:r0 + n, :] = x1
            f = _fold8(x1)
            acc = f if acc is None else acc + f
            z = yield acc
        mu = jnp.sum(acc, axis=0, keepdims=True) * (1.0 / D)
        src = lambda r0, n: o32[b, r0:r0 + n, :]
        rstd, z = yield from var_stages(src, mu, z)
        racc = None
        for ch in range(NCH):
            r0 = ch * CH
            x1 = src(r0, CH)
            h2 = (x1 - gate(mu, z)) * rstd * mcol(4, r0, CH) + mcol(3, r0, CH)
            o = x1 + mcol(5, r0, CH) * h2
            o32[b, r0:r0 + CH, :] = o
            obf[b, r0:r0 + CH, :] = o.astype(BF16)
            h2s[b, r0:r0 + CH, :] = h2.astype(BF16)
            f = _fold8(h2 * mcol(6, r0, CH))
            racc = f if racc is None else racc + f
            if ch == NCH - 1:
                rbuf[pl.ds(b, 1), :] = jnp.sum(racc, axis=0, keepdims=True)
            z = yield racc + o[CH - 8:]

    side = Side(ln1_stages(0))
    fuse_vo(NPAIR - 2, side)
    fuse_vo(NPAIR - 1, side)

    lane8 = jax.lax.broadcasted_iota(jnp.int32, (8, 128), 1)
    lo_half = lane8 < 64
    lane40 = jax.lax.broadcasted_iota(jnp.int32, (40, 128), 1)
    row40 = jax.lax.broadcasted_iota(jnp.int32, (40, 128), 0)
    lgrp40 = lane40 >> 4
    lgrp24 = jax.lax.broadcasted_iota(jnp.int32, (24, 128), 1) >> 4
    qpos = jnp.where(row40 < 8, SEG, (4 - (row40 >> 3)) * 8 + (row40 & 7))

    def proj_unit(lhs, w_s, buf, p, t, dests):
        if t < 3:
            r_e = jnp.dot(lhs, ldw(w_s, p * NT + t), preferred_element_type=F32)
            r_o = jnp.dot(lhs, ldw(w_s, p * NT + 4 + t), preferred_element_type=F32)
        else:
            r3 = jnp.dot(lhs, ldw(w_s, p * NT + 3), preferred_element_type=F32)
            lo = jax.lax.broadcasted_iota(jnp.int32, r3.shape, 1) < 64
            r_e, r_o = jnp.where(lo, r3, 0.0), jnp.where(lo, 0.0, r3)
        for g, (slot, jhi) in enumerate(dests):
            base = jhi * 64 + p * 8
            buf[slot, t, base:base + 8, :] = _pack2(r_e[8 * g:8 * g + 8],
                                                    r_o[8 * g:8 * g + 8])
        return r_e[0:8]

    UNITS = [(p, t) for t in range(4) for p in range(NPAIR)]

    def step(groups, dests, xq, mem_main, mem_tail, slot, side=None, zprev=None):
        first = zprev is None
        lhs = [jnp.concatenate([mem_main if g is None else g[:, :DM] for g in groups],
                               axis=0).astype(BF16)]

        def proj(w_s, buf, units):
            for i in range(0, len(units), 4):
                dep = side.stage() if side is not None else None
                res = [proj_unit(lhs[0], w_s, buf, p, t, dests) for p, t in units[i:i + 4]]
                if side is not None:
                    side.after(res[0])
                if dep is not None:
                    lhs[0] = tie(lhs[0], dep)

        proj(wg_s, gbuf, UNITS[:4])
        m3 = mem_tail()
        proj(wg_s, gbuf, UNITS[4:12])
        m3 = m3 + pltpu.roll(m3, 64, 1)
        ltail = jnp.concatenate([m3 if g is None else g[:, DM:] for g in groups],
                                axis=0).astype(BF16)
        lfull = jnp.concatenate([lhs[0], ltail[:, :64]], axis=1)
        for p in range(NPAIR):
            y = jnp.dot(lfull, ldw(wy_s, p), preferred_element_type=F32)
            for g, (sl, jhi) in enumerate(dests):
                ybuf[sl, p, (4 - jhi) * 8:(5 - jhi) * 8, :] = y[8 * g:8 * g + 8]
        proj(wg_s, gbuf, UNITS[12:16])
        memq = jnp.concatenate([mem_main, m3], axis=1)
        qf = jnp.concatenate([memq, xq[24:32], xq[16:24], xq[8:16], xq[0:8]], axis=0)
        q = qf.astype(BF16)
        tt = []
        for jhi in range(5):
            kt = qf[(4 - jhi) * 8:(5 - jhi) * 8, DM:]
            tt.append(_pack2(jnp.where(lo_half, kt, 0.0), jnp.where(lo_half, 0.0, kt)))
        tt = tt + [jnp.zeros((8, 128), U32)] * 3

        def tt_rot(pp):
            return bf(jnp.concatenate([tt[(l - pp) % 8] for l in range(8)], axis=0))

        rot = []
        for c in range(NPAIR // 2):
            ys = jnp.concatenate([ybuf[slot, 2 * c], ybuf[slot, 2 * c + 1]], axis=0)
            s2 = tdot(ys.astype(BF16), tt_rot(0))
            for i in range(2):
                pp = 2 * c + i
                blk = s2[40 * i:40 * i + 40]
                rot.append(blk if pp == 0 else pltpu.roll(blk, 16 * pp, 1))
        proj(wg_s, gbuf, UNITS[16:])
        proj(wu_s, ubuf, UNITS[:4])
        gmat = jnp.concatenate([bf(gbuf[slot, t]) for t in range(4)], axis=1)
        if first:
            st = []
            for jhi in range(5):
                st.append(tdot(q, gmat[jhi * 128:(jhi + 1) * 128]))
                if jhi < 4:
                    proj_unit(lhs[0], wu_s, ubuf, *UNITS[4 + jhi], dests)
            s = jnp.concatenate(st, axis=1)
            urest = UNITS[8:24]
        else:
            s = tdot(q, gmat)
            urest = UNITS[4:]
        sj = []
        for jhi in range(5):
            mrg = rot[NPAIR - 1]
            for pp in range(NPAIR - 2, -1, -1):
                mrg = jnp.where(lgrp40 == (jhi + pp) % 8, rot[pp], mrg)
            if jhi > 0:
                mrg = pltpu.roll(mrg, 128 - 16 * jhi, 1)
            blk = s[:, jhi * 128:(jhi + 1) * 128] + mrg
            if jhi < 4:
                key = jhi * 8 + ((lane40 >> 1) & 7)
                blk = jnp.where(qpos >= key, blk, -1000000000.0)
            sj.append(blk)
        m = functools.reduce(jnp.maximum, sj)
        m = _key_allreduce(m, jnp.maximum, lane40)
        ej = [jnp.exp(b - m) for b in sj]
        den = functools.reduce(jnp.add, ej)
        den = _key_allreduce(den, jnp.add, lane40)
        inv = 1.0 / den
        zrow = jnp.zeros((8, 128), F32)
        pj = [jnp.concatenate([e * inv, zrow], axis=0).astype(BF16) for e in ej]
        p_all = jnp.concatenate([pj[0], pj[4]], axis=1)
        p_top = jnp.concatenate([pj[1][:32], pj[2][:32], pj[3][:32]], axis=1)
        prot = [pltpu.bitcast(pj[0], U32)] + [
            pltpu.roll(pltpu.bitcast(pj[jhi], U32), 16 * jhi, 1) for jhi in range(1, 5)]
        proj(wu_s, ubuf, urest)
        z2 = []
        for pp in range(NPAIR):
            gat = prot[0]
            for jhi in range(1, 5):
                gat = jnp.where(lgrp24 == (jhi + pp) % 8, prot[jhi], gat)
            z2.append(jnp.dot(bf(gat), tt_rot(pp), preferred_element_type=F32))
        z2 = jnp.concatenate(z2, axis=1)
        if first:
            zl = z2[:32].astype(BF16)
        else:
            zl = jnp.concatenate([z2[:40], zprev], axis=0).astype(BF16)

        def pv(t):
            u = bf(ubuf[slot, t])
            o1 = jnp.dot(p_all, jnp.concatenate([u[0:128], u[512:640]], axis=0),
                         preferred_element_type=F32)
            o2 = jnp.dot(p_top, u[128:512], preferred_element_type=F32)
            return jnp.concatenate([o1[:32] + o2, o1[32:40]], axis=0)

        def zb(t):
            return jnp.dot(zl, ldw(wb_s, t), preferred_element_type=F32)

        def comb(o, o3):
            return jnp.concatenate([o[:32] + o3, o[32:]], axis=0) if first else o + o3[:40]

        o = jnp.concatenate([pv(t) for t in range(3)], axis=1)
        o3 = jnp.concatenate([zb(t) for t in range(3)], axis=1)
        if first:
            proj(wu_s, ubuf, UNITS[24:])
            o3t = zb(3)
            return comb(o, o3), (lambda: comb(pv(3), o3t)), z2[32:40]
        ot = pv(3)
        o3t = zb(3)
        return (comb(o, o3), comb(ot, o3t),
                jnp.concatenate([o3[40:48], o3t[40:48]], axis=1))

    def out_copy(b):
        return pltpu.make_async_copy(obf.at[b], out_hbm.at[:, pl.ds(b * TB, TB)], sem_o.at[b])

    abuf[...] = jnp.zeros((TB, DP), F32)

    def out_start(b):
        pltpu.make_async_copy(
            obf.at[b], out_hbm.at[:, pl.ds(pl.multiple_of(b * TB, TB), TB)],
            sem_o.at[b]).start()

    def x_wait(b):
        pltpu.make_async_copy(
            xt_hbm.at[:, pl.ds(pl.multiple_of(b * TB, TB), TB)], xs.at[b],
            sem_x.at[b]).wait()

    def pair_body(i, mem):
        @pl.when(i >= 2)
        def _():
            out_start(2 * i - 3)

        @pl.when(i >= 1)
        def _():
            out_start(2 * i - 2)

        x_wait(2 * i + 1)

        @pl.when(i < NBLK // 2 - 1)
        def _():
            x_wait(2 * i + 2)

        return blk_body(2 * i + 1, blk_body(2 * i, mem))

    def blk_body(t, mem):
        side_o = Side(out_stages(jnp.maximum(t - 1, 0)))
        side_l = Side(ln1_stages(jnp.minimum(t + 1, NBLK - 1)))
        for half in range(2):
            r0 = half * 64
            xa = hbuf[t, r0:r0 + SEG, :]
            xb = hbuf[t, r0 + SEG:r0 + 2 * SEG, :]
            ga_ = [xa[8 * g:8 * g + 8] for g in range(4)]
            gb_ = [xb[8 * g:8 * g + 8] for g in range(4)]
            side_l.budget = 8
            oa, oa_tail, zdef = step(
                ga_ + [None, gb_[3]], [(0, 0), (0, 1), (0, 2), (0, 3), (0, 4), (1, 3)],
                xa, mem[:, :DM], functools.partial(lambda m: m[:, DM:], mem), 0,
                side_o if half == 0 else side_l)
            cell = []

            def tail_a():
                cell.append(oa_tail())
                return cell[0][0:8]

            ob, ob_t, odef = step(
                gb_[:3] + [None], [(1, 0), (1, 1), (1, 2), (1, 4)],
                xb, oa[0:8], tail_a, 1, side_l if half == 0 else None, zdef)
            oa = jnp.concatenate([oa, cell[0]], axis=1)
            ob = jnp.concatenate([ob, ob_t], axis=1)
            mem = ob[0:8]
            abuf[r0:r0 + 8, :] = oa[32:40] + odef
            for g in range(1, 4):
                abuf[r0 + 8 * g:r0 + 8 * g + 8, :] = oa[32 - 8 * g:40 - 8 * g]
            for g in range(4):
                abuf[r0 + SEG + 8 * g:r0 + SEG + 8 * g + 8, :] = ob[32 - 8 * g:40 - 8 * g]
        return mem

    m0 = mem0_ref[...].astype(F32)
    mem0 = jnp.concatenate([m0, jnp.zeros((NM, 64), F32)], axis=1)
    jax.lax.fori_loop(0, NBLK // 2, pair_body, mem0)
    out_copy(NBLK - 3).start()
    out_copy(NBLK - 2).start()
    for _ in out_stages(NBLK - 1):
        pass
    out_copy(NBLK - 1).start()

    for cp in f_cp:
        cp.wait()
    rb = rbuf[...]
    rmax = jnp.max(jnp.max(rb, axis=0, keepdims=True), axis=1, keepdims=True)
    tok = (jax.lax.broadcasted_iota(jnp.int32, (NBLK, TB), 0) * TB
           + jax.lax.broadcasted_iota(jnp.int32, (NBLK, TB), 1))
    idx = jnp.min(jnp.where(rb == rmax, tok, S - 1))
    bsel = idx // TB
    lsel = idx - bsel * TB
    onehot = (jax.lax.broadcasted_iota(jnp.int32, (16, TB), 1) == lsel)
    onehot = jnp.where(onehot, 1.0, 0.0).astype(BF16)
    hsel = tdot(onehot, h2s[bsel]).astype(BF16)
    gate = jnp.dot(hsel, wgate_s[...], preferred_element_type=F32)
    up = jnp.dot(hsel, wup_s[...], preferred_element_type=F32)
    act = (gate * jax.nn.sigmoid(gate) * up)[0:1]
    rsel = jax.lax.broadcasted_iota(jnp.int32, (TB, FF), 0) == lsel
    actm = jnp.where(rsel, jnp.broadcast_to(act, (TB, FF)), 0.0).astype(BF16)
    yt = tdot(wdt_s[...], actm)
    yt = yt * jax.nn.sigmoid(rmax)
    for b in range(NBLK):
        out_copy(b).wait()
    obf[bsel] = (o32[bsel] + modt[5 * D:6 * D, :] * yt).astype(BF16)
    fix = pltpu.make_async_copy(
        obf.at[bsel], out_hbm.at[:, pl.ds(pl.multiple_of(bsel * TB, TB), TB)], sem_o.at[0])
    fix.start()
    fix.wait()


@jax.jit
def _run(A_x, A_mem0, A_Wq, A_Wk, A_Wv, A_Wo, B_w_r, B_w_gate, B_w_up, B_w_down, c, w_mod):
    xt = jnp.transpose(A_x.reshape(S, D))
    mem0 = A_mem0.reshape(NM, D)
    wq = A_Wq.reshape(D * H, DH)
    wk = A_Wk.reshape(D * H, DH)
    wv = A_Wv.reshape(D * H, DH)
    wot = jnp.transpose(A_Wo, (0, 2, 1))
    wdt = jnp.transpose(B_w_down)
    vmem = pl.BlockSpec(memory_space=pltpu.VMEM)
    hbm = pl.BlockSpec(memory_space=pl.ANY)
    out_t = pl.pallas_call(
        _kernel,
        out_shape=jax.ShapeDtypeStruct((D, S), BF16),
        in_specs=[hbm, vmem, hbm, hbm, hbm, hbm, vmem, hbm, hbm, hbm, vmem, hbm],
        out_specs=hbm,
        scratch_shapes=[
            pltpu.VMEM((6, D * H, 128), BF16),
            pltpu.VMEM((H, D, DH), BF16),
            pltpu.VMEM((D, 6 * D), BF16),
            pltpu.VMEM((D, FF), BF16),
            pltpu.VMEM((D, FF), BF16),
            pltpu.VMEM((D, FF), BF16),
            pltpu.VMEM((NBLK, D, TB), BF16),
            pltpu.VMEM((NPAIR * NT, DM, 128), BF16),
            pltpu.VMEM((NPAIR * NT, DM, 128), BF16),
            pltpu.VMEM((25 * 128, 128), F32),
            pltpu.VMEM((NBLK, TB, DP), F32),
            pltpu.VMEM((TB, DP), F32),
            pltpu.VMEM((2, 4, 320, 128), U32),
            pltpu.VMEM((2, 4, 320, 128), U32),
            pltpu.VMEM((NBLK, D, TB), F32),
            pltpu.VMEM((NBLK, D, TB), BF16),
            pltpu.VMEM((NBLK, D, TB), BF16),
            pltpu.VMEM((NBLK, TB), F32),
            pltpu.VMEM((3 * H * 2, D, 128), BF16),
            pltpu.VMEM((NPAIR, D, 128), BF16),
            pltpu.VMEM((4, NPAIR * 128, 128), BF16),
            pltpu.VMEM((2, NPAIR, 40, 128), F32),
            pltpu.SMEM((1,), jnp.int32),
            pltpu.SemaphoreType.DMA((16,)),
            pltpu.SemaphoreType.DMA((NBLK,)),
            pltpu.SemaphoreType.DMA((3,)),
            pltpu.SemaphoreType.DMA((NBLK,)),
        ],
        compiler_params=pltpu.CompilerParams(vmem_limit_bytes=110 * 1024 * 1024),
    )(xt, mem0, wq, wk, wv, wot, B_w_r, B_w_gate, B_w_up, wdt, c, w_mod)
    return jnp.transpose(out_t).reshape(1, S, D)


def pallas_adaLN_cond__memory_aug_recurrent_mem_tr__moe_arch_mod__prompt_kernel(
    A_x, A_mem0, A_Wq, A_Wk, A_Wv, A_Wo, A_seg_len, B_x, B_w_r, B_w_gate, B_w_up,
    B_w_down, c, w_mod,
):
    del A_seg_len, B_x
    return _run(A_x, A_mem0, A_Wq, A_Wk, A_Wv, A_Wo, B_w_r, B_w_gate, B_w_up, B_w_down,
                c, w_mod)
```

```python
import functools

import jax
import jax.numpy as jnp
import jax.experimental.pallas as pl
import jax.experimental.pallas.tpu as pltpu

F32 = jnp.float32
BF16 = jnp.bfloat16
U32 = jnp.uint32

S = 2048
D = 448
DM = 384
DP = 512
H = 16
DH = 256
NM = 8
SEG = 32
FF = 1792
NPAIR = H // 2
NT = 7
TB = 128
NBLK = S // TB
EPS = 1e-5
CH = 64
NCH = D // CH
SPEC = frozenset((17, 18, 19, 20, 21, 33, 34, 35))
SCHED_A = {21: [(0, (0, 1))], 22: [(1, (0, 1))], 23: [(2, (0, 1))], 24: [(3, (0, 1))],
           25: [(4, (0, 1))], 35: [(0, (2, 3))], 36: [(1, (2, 3))], 37: [(2, (2, 3))],
           38: [(3, (2, 3))], 39: [(4, (2, 3))]}
SCHED_B = {17: [(0, (0, 1))], 18: [(1, (0, 1))], 19: [(2, (0, 1))], 20: [(3, (0, 1))],
           21: [(4, (0, 1))], 34: [(0, (2, 3)), (1, (2, 3))],
           35: [(2, (2, 3)), (3, (2, 3))], 36: [(4, (2, 3))]}
TDIMS = (((1,), (1,)), ((), ()))


def _key_allreduce(v, op, lane):
    for k in (1, 2, 4):
        up = pltpu.roll(v, k, 1)
        dn = pltpu.roll(v, 128 - k, 1)
        v = op(v, jnp.where((lane & k) != 0, up, dn))
    return v


def _fold8(v):
    acc = v[0:8]
    for i in range(1, v.shape[0] // 8):
        acc = acc + v[8 * i:8 * i + 8]
    return acc


def _kernel(xt_hbm, mem0_hbm, wq_hbm, wk_hbm, wv_hbm, wot_hbm, wr_hbm, wgate_hbm,
            wup_hbm, wdt_hbm, c_hbm, wmod_hbm, out_hbm,
            wraw, wot_s, wmod_s, wgate_s, wup_s, wdt_s, xs, wg_s, wu_s, modt, hbuf,
            abuf, gbuf, ubuf, o32, obf, h2s, rbuf, hx, wy_s, wb_s, ybuf, ttbuf,
            mem0_ref, wr_ref, c_ref, zsm,
            sem_w, sem_x, sem_f, sem_o):
    def half_copies(w_hbm, wi, r0, nrows, s0):
        return [pltpu.make_async_copy(w_hbm.at[pl.ds(r0, nrows), pl.ds(e * 128, 128)],
                                      wraw.at[wi * 2 + e, pl.ds(r0, nrows)],
                                      sem_w.at[s0 + e]) for e in range(2)]
    KH = D // 2
    k_cp = [half_copies(wk_hbm, 1, 0, KH * H, 0), half_copies(wk_hbm, 1, KH * H, KH * H, 2)]
    q_cp = [half_copies(wq_hbm, 0, 0, 128 * H, 4),
            half_copies(wq_hbm, 0, 128 * H, 128 * H, 6),
            half_copies(wq_hbm, 0, 256 * H, 192 * H, 8)]
    VCH = ((0, 160), (160, 320), (320, 448))
    v_cp = [half_copies(wv_hbm, 2, a * H, (b - a) * H, sm)
            for (a, b), sm in zip(VCH, (10, 20, 22))]
    o_cp = [pltpu.make_async_copy(wot_hbm.at[pl.ds(h0, nh)], wot_s.at[pl.ds(h0, nh)],
                                  sem_w.at[12 + i])
            for i, (h0, nh) in enumerate(((0, 6), (6, 6), (12, 4)))]
    mod_cp = [pltpu.make_async_copy(wmod_hbm.at[:, pl.ds(c0, nc)],
                                    wmod_s.at[:, pl.ds(c0, nc)], sem_w.at[15 + i])
              for i, (c0, nc) in enumerate(((0, 2 * D), (2 * D, 4 * D)))]
    x_cp = [pltpu.make_async_copy(xt_hbm.at[:, pl.ds(b * TB, TB)], xs.at[b], sem_x.at[b])
            for b in range(NBLK)]
    f_cp = [pltpu.make_async_copy(src, dst, sem_f.at[i]) for i, (src, dst) in
            enumerate(((wgate_hbm, wgate_s), (wup_hbm, wup_s), (wdt_hbm, wdt_s)))]
    s_cp = [pltpu.make_async_copy(src, dst, sem_w.at[17 + i]) for i, (src, dst) in
            enumerate(((mem0_hbm, mem0_ref), (wr_hbm, wr_ref), (c_hbm, c_ref)))]
    for cp in (k_cp[0] + q_cp[0] + k_cp[1] + s_cp + q_cp[1] + q_cp[2] + o_cp[:1]
               + v_cp[0] + v_cp[1] + v_cp[2]
               + [o_cp[1], x_cp[0], mod_cp[0], o_cp[2], mod_cp[1]]):
        cp.start()
    zsm[0] = 0

    def bf(v):
        return pltpu.bitcast(v, BF16)

    def ldw(ref, n, r0=0, r1=None):
        r1 = ref.shape[1] if r1 is None else r1
        return bf(ref.bitcast(U32)[n, r0 // 2:r1 // 2, :])

    def heads(wi, hp, d0=0, nd=D, mul=None):
        for e in range(2):
            w32 = wraw.at[wi * 2 + e].bitcast(U32)
            v = w32[pl.ds(d0 * 8 + hp, nd, stride=8), :]
            lo = pltpu.bitcast(v << 16, F32)
            hi = pltpu.bitcast(v & jnp.uint32(0xFFFF0000), F32)
            if mul is not None:
                lo, hi = lo * mul, hi * mul
            hx[(wi * H + 2 * hp) * 2 + e, d0:d0 + nd, :] = lo.astype(BF16)
            hx[(wi * H + 2 * hp + 1) * 2 + e, d0:d0 + nd, :] = hi.astype(BF16)

    def head(wi, h, d0=0, nd=D):
        return jnp.concatenate([ldw(hx, (wi * H + h) * 2 + e, d0, d0 + nd)
                                for e in range(2)], axis=1)

    z64 = jnp.zeros((64, DH), BF16)

    def tdot(a, b):
        return jax.lax.dot_general(a, b, TDIMS, preferred_element_type=F32)

    def zmask(dep):
        return pltpu.bitcast(dep, jnp.int32) & jnp.full((8, 128), zsm[0], jnp.int32)

    def tie(lhs, dep):
        l32 = pltpu.bitcast(lhs, jnp.int32)
        top = jnp.concatenate([l32[0:8, 0:128] | zmask(dep), l32[0:8, 128:]], axis=1)
        return pltpu.bitcast(jnp.concatenate([top, l32[8:]], axis=0), BF16)

    def gate(v, z):
        if z is None:
            return v
        zz = z[0:1] if v.shape[0] == 1 else jnp.concatenate([z] * (v.shape[0] // 8), axis=0)
        return pltpu.bitcast(pltpu.bitcast(v, jnp.int32) | zz, F32)

    class Side:
        def __init__(self, gen):
            self.gen, self.started, self.z, self.budget = gen, False, None, 1000

        def stage(self):
            if self.gen is None or self.budget == 0:
                return None
            self.budget -= 1
            try:
                if not self.started:
                    self.started = True
                    next(self.gen)
                return self.gen.send(self.z)
            except StopIteration:
                self.gen = None
                return None

        def after(self, res):
            self.z = zmask(res) if self.gen is not None else None

    scale = float(DH) ** -0.5

    pending = []

    def flush():
        while pending:
            pending.pop()()

    def a_tiles(p, j, r0, r1):
        a_e = tdot(head(1, 2 * p, r0, r1 - r0), head(0, 2 * p, j * 128, 128))
        a_o = tdot(head(1, 2 * p + 1, r0, r1 - r0), head(0, 2 * p + 1, j * 128, 128))
        rm = min(r1, DM)
        wg_s[p * NT + j, r0:rm, :] = a_e[:rm - r0].astype(BF16)
        wg_s[p * NT + 4 + j, r0:rm, :] = a_o[:rm - r0].astype(BF16)
        flush()
        if r1 > DM:
            def fin():
                wy = jnp.concatenate([a_e[DM - r0:], a_o[DM - r0:]], axis=0).T
                wy_s[p, j * 128:(j + 1) * 128, :] = wy.astype(BF16)
            pending.append(fin)

    def tail_t(l_e, l_o, r_e, r_o):
        t_e = tdot(l_e, jnp.concatenate([r_e, z64], axis=0))
        t_o = tdot(l_o, jnp.concatenate([r_o[:DM], z64, r_o[DM:]], axis=0))
        return t_e, t_o

    for half in range(2):
        for cp in k_cp[half] + (q_cp[0] if half == 0 else []):
            cp.wait()
        for p in range(NPAIR):
            heads(1, p, half * KH, KH)
            if half == 0:
                heads(0, p, 0, 128, scale)
            a_tiles(p, 0, half * KH, (half + 1) * KH)
    for j in (1, 2):
        for cp in q_cp[j]:
            cp.wait()
        for p in range(NPAIR):
            heads(0, p, j * 128, 128, scale)
            a_tiles(p, j, 0, D)
    for p in range(NPAIR):
        heads(0, p, DM, 64, scale)
        t_e, t_o = tail_t(head(0, 2 * p, DM, 64), head(0, 2 * p + 1, DM, 64),
                          head(1, 2 * p), head(1, 2 * p + 1))
        flush()

        def fin(p=p, t_e=t_e, t_o=t_o):
            for i in range(3):
                blk = jnp.concatenate([t_e[:, i * 128:(i + 1) * 128],
                                       t_o[:, i * 128:(i + 1) * 128]], axis=0).T
                wg_s[p * NT + 3, i * 128:(i + 1) * 128, :] = blk.astype(BF16)
        pending.append(fin)
        wy = (t_e[:, DM:] + t_o[:, DM:]).astype(BF16)
        wy_s[p, DM:D, :] = wy

    def fuse_vo(p, side=None, extra=None, b0=0, b1=D):
        heads(2, p, b0, b1 - b0)
        v_e, v_o = head(2, 2 * p, b0, b1 - b0), head(2, 2 * p + 1, b0, b1 - b0)
        r_e, r_o = wot_s[2 * p], wot_s[2 * p + 1]
        bm = min(b1, DM)
        for t in ((0, 1, 3, 2, 4, 5, 6) if b1 == D else (0, 1, 2, 4, 5, 6)):
            if extra is not None and t in (3, 2, 5):
                next(extra, None)
            dep = side.stage() if side is not None else None
            if t == 3:
                t_e, t_o = tail_t(r_e[DM:], r_o[DM:], head(2, 2 * p), head(2, 2 * p + 1))
                for i in range(4):
                    blk = jnp.concatenate([t_e[:, i * 128:(i + 1) * 128],
                                           t_o[:, i * 128:(i + 1) * 128]], axis=0).T
                    if i < 3:
                        wu_s[p * NT + 3, i * 128:(i + 1) * 128, :] = blk.astype(BF16)
                    else:
                        wb_s[3, p * 128:(p + 1) * 128, :] = blk.astype(BF16)
                res = t_e[0:8, 0:128]
            else:
                tv = (tdot(v_e, r_e[t * 128:(t + 1) * 128]) if t < 3
                      else tdot(v_o, r_o[(t - 4) * 128:(t - 3) * 128]))
                wu_s[p * NT + t, b0:bm, :] = tv[:bm - b0].astype(BF16)
                if b1 == D:
                    r0 = p * 128 + (64 if t > 3 else 0)
                    wb_s[t % 4, r0:r0 + 64, :] = tv[DM - b0:].astype(BF16)
                res = tv[0:8]
            if side is not None:
                side.after(res)
            if dep is not None:
                v_e, v_o = tie(v_e, dep), tie(v_o, dep)

    for i, (a, b) in enumerate(VCH):
        for cp in (s_cp + o_cp[:1] if i == 0 else []) + v_cp[i]:
            cp.wait()
        for p in range(3):
            fuse_vo(p, b0=a, b1=b)
            flush()
    o_cp[1].wait()
    for p in (3, 4, 5):
        fuse_vo(p)

    cvec = c_ref[...].astype(F32)
    sc = cvec * jax.nn.sigmoid(cvec)
    sc = jnp.broadcast_to(sc, (16, D)).astype(BF16)

    def bcast_cols(row, i0):
        for i in range(row.shape[1] // 128):
            blk = jnp.broadcast_to(row[:, i * 128:(i + 1) * 128], (128, 128))
            modt[(i0 + i) * 128:(i0 + i + 1) * 128, :] = blk.T

    def mod_stages(t0, t1, nt):
        for i0 in range(t0, t1, nt):
            c0, c1 = i0 * 128, min(i0 + nt, t1) * 128
            mod = jnp.dot(sc, wmod_s[:, c0:c1], preferred_element_type=F32)[0:1]
            mod = mod.astype(BF16).astype(F32)
            col = c0 + jax.lax.broadcasted_iota(jnp.int32, mod.shape, 1)
            is_scale = ((col >= D) & (col < 2 * D)) | ((col >= 4 * D) & (col < 5 * D))
            mod1 = (1.0 + mod).astype(BF16).astype(F32)
            bcast_cols(jnp.where(is_scale, mod1, mod), i0)
            yield

    wr = wr_ref[...].astype(F32).reshape(1, D)
    bcast_cols(jnp.concatenate([wr, jnp.zeros((1, 64), F32)], axis=1), 21)

    def mcol(i, r0, n):
        return modt[i * D + r0:i * D + r0 + n, :]

    TILES = ((0, 128), (128, 128), (256, 128), (384, 64))

    def rb16(v):
        return v.astype(BF16).astype(F32)

    def var_stages(src, mu, z):
        acc = None
        for r0, n in TILES:
            xc = src(r0, n) - gate(mu, z)
            f = _fold8(xc * xc)
            acc = f if acc is None else acc + f
            z = yield acc
        var = jnp.sum(acc, axis=0, keepdims=True) * (1.0 / D)
        return 1.0 / rb16(jnp.sqrt(rb16(rb16(var) + EPS))), z

    def ln1_stages(b):
        src = lambda r0, n: xs[b, r0:r0 + n, :].astype(F32)
        z = yield
        acc = None
        for r0, n in TILES:
            f = _fold8(gate(src(r0, n), z))
            acc = f if acc is None else acc + f
            z = yield acc
        mu = jnp.sum(acc, axis=0, keepdims=True) * (1.0 / D)
        rstd, z = yield from var_stages(src, mu, z)
        mu = rb16(mu)
        for t, (r0, n) in enumerate(TILES):
            ht = (src(r0, n) - gate(mu, z)) * rstd * mcol(1, r0, n) + mcol(0, r0, n)
            if n == 64:
                ht = jnp.concatenate([ht, ht], axis=0)
            tile = ht.T
            hbuf[b, :, t * 128:(t + 1) * 128] = tile
            z = yield tile[120:128]

    def out_stages(b):
        z = yield
        acc = None
        for t, (r0, n) in enumerate(TILES):
            a = gate(abuf[:, t * 128:(t + 1) * 128], z).T
            if n == 64:
                a = a[:64] + a[64:]
            x1 = xs[b, r0:r0 + n, :].astype(F32) + mcol(2, r0, n) * a
            o32[b, r0:r0 + n, :] = x1
            f = _fold8(x1)
            acc = f if acc is None else acc + f
            z = yield acc
        mu = jnp.sum(acc, axis=0, keepdims=True) * (1.0 / D)
        src = lambda r0, n: o32[b, r0:r0 + n, :]
        rstd, z = yield from var_stages(src, mu, z)
        mu = rb16(mu)
        racc = None
        for ch in range(NCH):
            r0 = ch * CH
            x1 = src(r0, CH)
            h2 = (x1 - gate(mu, z)) * rstd * mcol(4, r0, CH) + mcol(3, r0, CH)
            o = x1 + mcol(5, r0, CH) * h2
            o32[b, r0:r0 + CH, :] = o
            obf[b, r0:r0 + CH, :] = o.astype(BF16)
            h2s[b, r0:r0 + CH, :] = h2.astype(BF16)
            f = _fold8(h2 * mcol(6, r0, CH))
            racc = f if racc is None else racc + f
            if ch == NCH - 1:
                rbuf[pl.ds(b, 1), :] = rb16(jnp.sum(racc, axis=0, keepdims=True))
            z = yield racc + o[CH - 8:]

    x_cp[0].wait()
    mod_cp[0].wait()
    o_cp[2].wait()
    for cp in x_cp[1:3]:
        cp.start()
    side = Side(ln1_stages(0))
    fuse_vo(NPAIR - 2, side, mod_stages(0, 7, 3))
    mod_cp[1].wait()
    for cp in x_cp[3:]:
        cp.start()
    fuse_vo(NPAIR - 1, side, mod_stages(7, 21, 5))

    lane8 = jax.lax.broadcasted_iota(jnp.int32, (8, 128), 1)
    lo_half = lane8 < 64
    lane40 = jax.lax.broadcasted_iota(jnp.int32, (40, 128), 1)
    lgrp24 = jax.lax.broadcasted_iota(jnp.int32, (24, 128), 1) >> 4

    def proj_unit(lhs, w_s, buf, p, t, dests):
        if t < 3:
            r_e = jnp.dot(lhs, ldw(w_s, p * NT + t), preferred_element_type=F32)
            r_o = jnp.dot(lhs, ldw(w_s, p * NT + 4 + t), preferred_element_type=F32)
        else:
            r3 = jnp.dot(lhs, ldw(w_s, p * NT + 3), preferred_element_type=F32)
            lo = jax.lax.broadcasted_iota(jnp.int32, r3.shape, 1) < 64
            r_e, r_o = jnp.where(lo, r3, 0.0), jnp.where(lo, 0.0, r3)
        for g, (slot, jhi) in enumerate(dests):
            base = jhi * 128 + p * 16
            buf[slot * 4 + t, base:base + 16, :] = jnp.concatenate(
                [r_e[8 * g:8 * g + 8], r_o[8 * g:8 * g + 8]], axis=0).astype(BF16)
        return r_e[0:8]

    UNITS = [(p, t) for t in range(4) for p in range(NPAIR)]

    def step(groups, dests, xq, mem_main, mem_tail, slot, side=None, zprev=None,
             skip_mid=False, ahead=None):
        first = zprev is None
        lhs = [jnp.concatenate([mem_main if g is None else g[:, :DM] for g in groups],
                               axis=0).astype(BF16)]
        if ahead is not None:
            ext = jnp.concatenate([g[:, :DM] for g in ahead], axis=0).astype(BF16)
        NROW = (40, 32, 24, 16, 40)
        qx = jnp.concatenate([xq[24:32], xq[16:24], xq[8:16], xq[0:8]], axis=0)
        qt = [jnp.concatenate([mem_main[:, t * 128:(t + 1) * 128],
                               qx[:, t * 128:(t + 1) * 128]], axis=0).astype(BF16)
              for t in range(3)]
        st = [None] * 5
        sched = SCHED_A if first else SCHED_B
        state = {"n": 0, "dep": None}

        def score_pass(jhi, ts):
            nq = min(40, -(-NROW[jhi] // 16) * 16)
            a = jnp.concatenate([qt[t][:nq] for t in ts], axis=1)
            b = jnp.concatenate([ldw(gbuf, slot * 4 + t, jhi * 128, (jhi + 1) * 128)
                                 for t in ts], axis=1)
            r = tdot(a, b)[:NROW[jhi]]
            st[jhi] = r if st[jhi] is None else st[jhi] + r

        def run(u0, u1):
            for u in range(u0, u1):
                hook = side is not None and state["n"] % 4 == 0
                if hook:
                    if state["dep"] is not None:
                        lhs[0] = tie(lhs[0], state["dep"])
                    state["dep"] = side.stage()
                l_, d_ = lhs[0], dests
                if u in SPEC and skip_mid:
                    l_ = jnp.concatenate([l_[0:16], l_[32:48]], axis=0)
                    d_ = dests[:2] + dests[4:]
                elif u in SPEC and ahead is not None:
                    l_ = jnp.concatenate([l_, ext], axis=0)
                    d_ = dests + [(0, 3), (0, 2)]
                w_s, buf = (wg_s, gbuf) if u < 32 else (wu_s, ubuf)
                res = proj_unit(l_, w_s, buf, *UNITS[u % 32], d_)
                if hook:
                    side.after(res)
                state["n"] += 1
                for jhi, ts in sched.get(u, ()):
                    score_pass(jhi, ts)

        run(0, 4)
        m3 = mem_tail()
        run(4, 12)
        m3 = m3 + pltpu.roll(m3, 64, 1)
        ltail = jnp.concatenate([m3 if g is None else g[:, DM:] for g in groups],
                                axis=0).astype(BF16)
        lfull = jnp.concatenate([lhs[0], ltail[:, :64]], axis=1)
        for p in range(NPAIR):
            y = jnp.dot(lfull, ldw(wy_s, p), preferred_element_type=F32)
            for g, (sl, jhi) in enumerate(dests):
                ybuf[sl, p, (4 - jhi) * 8:(5 - jhi) * 8, :] = y[8 * g:8 * g + 8]
        run(12, 16)
        qf3 = jnp.concatenate([m3, qx[:, DM:]], axis=0)
        qt.append(qf3.astype(BF16))
        for jhi in range(5):
            kt = qf3[(4 - jhi) * 8:(5 - jhi) * 8]
            ttbuf[slot, jhi * 16:(jhi + 1) * 16, :] = jnp.concatenate(
                [jnp.where(lo_half, kt, 0.0), jnp.where(lo_half, 0.0, kt)],
                axis=0).astype(BF16)
        tt32 = ttbuf.bitcast(U32)
        tt = [tt32[slot, jhi * 8:(jhi + 1) * 8, :] for jhi in range(5)]
        tt = tt + [jnp.zeros((8, 128), U32)] * 3

        def tt_rot(pp):
            return bf(jnp.concatenate([tt[(l - pp) % 8] for l in range(8)], axis=0))

        rot = []
        for c in range(NPAIR // 2):
            ys = jnp.concatenate([ybuf[slot, 2 * c], ybuf[slot, 2 * c + 1]], axis=0)
            s2 = tdot(ys.astype(BF16), tt_rot(0))
            for i in range(2):
                pp = 2 * c + i
                blk = s2[40 * i:40 * i + 40]
                rot.append(blk if pp == 0 else pltpu.roll(blk, 16 * pp, 1))
        ulast = max(sched) + 1
        run(16, ulast)
        sj = []
        for jhi in range(5):
            n = NROW[jhi]
            lane_n = jax.lax.broadcasted_iota(jnp.int32, (n, 128), 1)
            mrg = rot[NPAIR - 1][:n]
            for pp in range(NPAIR - 2, -1, -1):
                mrg = jnp.where((lane_n >> 4) == (jhi + pp) % 8, rot[pp][:n], mrg)
            if jhi > 0:
                mrg = pltpu.roll(mrg, 128 - 16 * jhi, 1)
            blk = st[jhi] + mrg
            if jhi < 4:
                row_n = jax.lax.broadcasted_iota(jnp.int32, (n, 128), 0)
                qpos = jnp.where(row_n < 8, SEG, (4 - (row_n >> 3)) * 8 + (row_n & 7))
                blk = jnp.where(qpos >= jhi * 8 + (lane_n & 7), blk, -1000000000.0)
            sj.append(blk)

        def merge(vals, op):
            acc = op(vals[0], vals[4])
            for jhi in (1, 2, 3):
                n = NROW[jhi]
                acc = jnp.concatenate([op(acc[:n], vals[jhi]), acc[n:]], axis=0)
            return _key_allreduce(acc, op, lane40)

        m = merge(sj, jnp.maximum)
        ej = [jnp.exp(sj[jhi] - m[:NROW[jhi]]) for jhi in range(5)]
        inv = 1.0 / merge(ej, jnp.add)
        pj = [jnp.concatenate([ej[jhi] * inv[:NROW[jhi]],
                               jnp.zeros((48 - NROW[jhi], 128), F32)], axis=0).astype(BF16)
              for jhi in range(5)]
        p_all = jnp.concatenate([pj[0], pj[4]], axis=1)
        p_top = jnp.concatenate([pj[1][:32], pj[2][:32], pj[3][:32]], axis=1)
        prot = [pltpu.bitcast(pj[0], U32)] + [
            pltpu.roll(pltpu.bitcast(pj[jhi], U32), 16 * jhi, 1) for jhi in range(1, 5)]
        run(ulast, 56 if first else 64)
        z2 = []
        for pp in range(NPAIR):
            gat = prot[0]
            for jhi in range(1, 5):
                gat = jnp.where(lgrp24 == (jhi + pp) % 8, prot[jhi], gat)
            z2.append(jnp.dot(bf(gat), tt_rot(pp), preferred_element_type=F32))
        z2 = jnp.concatenate(z2, axis=1)
        if first:
            zl = z2[:32].astype(BF16)
        else:
            zl = jnp.concatenate([z2[:40], zprev], axis=0).astype(BF16)

        def pv(t):
            u = ldw(ubuf, slot * 4 + t)
            o1 = jnp.dot(p_all, jnp.concatenate([u[0:128], u[512:640]], axis=0),
                         preferred_element_type=F32)
            o2 = jnp.dot(p_top, u[128:512], preferred_element_type=F32)
            return jnp.concatenate([o1[:32] + o2, o1[32:40]], axis=0)

        def zb(t):
            return jnp.dot(zl, ldw(wb_s, t), preferred_element_type=F32)

        def comb(o, o3):
            return jnp.concatenate([o[:32] + o3, o[32:]], axis=0) if first else o + o3[:40]

        o = jnp.concatenate([pv(t) for t in range(3)], axis=1)
        o3 = jnp.concatenate([zb(t) for t in range(3)], axis=1)
        if first:
            run(56, 64)
            while side is not None and side.stage() is not None:
                pass
            o3t = zb(3)
            return comb(o, o3), (lambda: comb(pv(3), o3t)), z2[32:40]
        ot = pv(3)
        o3t = zb(3)
        return (comb(o, o3), comb(ot, o3t),
                jnp.concatenate([o3[40:48], o3t[40:48]], axis=1))

    def out_copy(b):
        return pltpu.make_async_copy(obf.at[b], out_hbm.at[:, pl.ds(b * TB, TB)], sem_o.at[b])

    abuf[...] = jnp.zeros((TB, DP), F32)

    def out_start(b):
        pltpu.make_async_copy(
            obf.at[b], out_hbm.at[:, pl.ds(pl.multiple_of(b * TB, TB), TB)],
            sem_o.at[b]).start()

    def x_wait(b):
        pltpu.make_async_copy(
            xt_hbm.at[:, pl.ds(pl.multiple_of(b * TB, TB), TB)], xs.at[b],
            sem_x.at[b]).wait()

    def pair_body(i, mem):
        @pl.when(i >= 2)
        def _():
            out_start(2 * i - 3)

        @pl.when(i >= 1)
        def _():
            out_start(2 * i - 2)

        @pl.when(i == 1)
        def _():
            for cp in f_cp:
                cp.start()

        x_wait(2 * i + 1)

        @pl.when(i < NBLK // 2 - 1)
        def _():
            x_wait(2 * i + 2)

        return blk_body(2 * i + 1, blk_body(2 * i, mem, 0), 1)

    def blk_body(t, mem, pos):
        side_o = Side(out_stages(jnp.maximum(t - 1, 0)))
        side_l = Side(ln1_stages(jnp.minimum(t + 1, NBLK - 1)))
        for half in range(2):
            r0 = half * 64
            xa = hbuf[t, r0:r0 + SEG, :]
            xb = hbuf[t, r0 + SEG:r0 + 2 * SEG, :]
            ga_ = [xa[8 * g:8 * g + 8] for g in range(4)]
            gb_ = [xb[8 * g:8 * g + 8] for g in range(4)]
            side_l.budget = 8
            oa, oa_tail, zdef = step(
                ga_ + [None, gb_[3]], [(0, 0), (0, 1), (0, 2), (0, 3), (0, 4), (1, 3)],
                xa, mem[:, :DM], functools.partial(lambda m: m[:, DM:], mem), 0,
                side_o if half == 0 else side_l, skip_mid=(pos, half) != (0, 0))
            if half == 0:
                nxt = hbuf[t, 64 + 16:64 + 32, :]
            elif pos == 0:
                nxt = hbuf[t + 1, 16:32, :]
            ahead = None if (pos, half) == (1, 1) else [nxt[8:16], nxt[0:8]]
            cell = []

            def tail_a():
                cell.append(oa_tail())
                return cell[0][0:8]

            ob, ob_t, odef = step(
                gb_[:3] + [None], [(1, 0), (1, 1), (1, 2), (1, 4)],
                xb, oa[0:8], tail_a, 1, side_l if half == 0 else None, zdef,
                ahead=ahead)
            oa = jnp.concatenate([oa, cell[0]], axis=1)
            ob = jnp.concatenate([ob, ob_t], axis=1)
            mem = ob[0:8]
            abuf[r0:r0 + 8, :] = oa[32:40] + odef
            for g in range(1, 4):
                abuf[r0 + 8 * g:r0 + 8 * g + 8, :] = oa[32 - 8 * g:40 - 8 * g]
            for g in range(4):
                abuf[r0 + SEG + 8 * g:r0 + SEG + 8 * g + 8, :] = ob[32 - 8 * g:40 - 8 * g]
        return mem

    m0 = mem0_ref[...].astype(F32)
    mem0 = jnp.concatenate([m0, jnp.zeros((NM, 64), F32)], axis=1)
    jax.lax.fori_loop(0, NBLK // 2, pair_body, mem0)
    out_copy(NBLK - 3).start()
    out_copy(NBLK - 2).start()
    for cp in f_cp:
        cp.wait()
    for b in range(NBLK - 3):
        out_copy(b).wait()
    for _ in out_stages(NBLK - 1):
        pass
    out_copy(NBLK - 1).start()

    rb = rbuf[...]
    rmax = jnp.max(jnp.max(rb, axis=0, keepdims=True), axis=1, keepdims=True)
    tok = (jax.lax.broadcasted_iota(jnp.int32, (NBLK, TB), 0) * TB
           + jax.lax.broadcasted_iota(jnp.int32, (NBLK, TB), 1))
    idx = jnp.min(jnp.where(rb == rmax, tok, S - 1))
    bsel = idx // TB
    lsel = idx - bsel * TB
    onehot = (jax.lax.broadcasted_iota(jnp.int32, (16, TB), 1) == lsel)
    onehot = jnp.where(onehot, 1.0, 0.0).astype(BF16)
    hsel = tdot(onehot, h2s[bsel]).astype(BF16)
    gv = jnp.dot(hsel, wgate_s[...], preferred_element_type=F32)
    uv = jnp.dot(hsel, wup_s[...], preferred_element_type=F32)
    act = (gv * jax.nn.sigmoid(gv) * uv).astype(BF16)
    y = tdot(act, wdt_s[...])[0:1] * jax.nn.sigmoid(rmax)
    y = jnp.concatenate([y, jnp.zeros((1, DP - D), F32)], axis=1)
    rsel = jax.lax.broadcasted_iota(jnp.int32, (TB, TB), 0) == lsel
    yt = jnp.concatenate(
        [jnp.where(rsel, jnp.broadcast_to(y[:, i * 128:(i + 1) * 128], (TB, 128)), 0.0).T
         for i in range(4)], axis=0)[:D]
    fixed = (o32[bsel] + modt[5 * D:6 * D, :] * yt).astype(BF16)
    for b in range(NBLK - 3, NBLK):
        out_copy(b).wait()
    obf[bsel] = fixed
    fix = pltpu.make_async_copy(
        obf.at[bsel], out_hbm.at[:, pl.ds(pl.multiple_of(bsel * TB, TB), TB)], sem_o.at[0])
    fix.start()
    fix.wait()


@jax.jit
def _run(A_x, A_mem0, A_Wq, A_Wk, A_Wv, A_Wo, B_w_r, B_w_gate, B_w_up, B_w_down, c, w_mod):
    xt = jnp.transpose(A_x.reshape(S, D))
    mem0 = A_mem0.reshape(NM, D)
    wq = A_Wq.reshape(D * H, DH)
    wk = A_Wk.reshape(D * H, DH)
    wv = A_Wv.reshape(D * H, DH)
    wot = jnp.transpose(A_Wo, (0, 2, 1))
    wdt = jnp.transpose(B_w_down)
    hbm = pl.BlockSpec(memory_space=pl.ANY)
    out_t = pl.pallas_call(
        _kernel,
        out_shape=jax.ShapeDtypeStruct((D, S), BF16),
        in_specs=[hbm] * 12,
        out_specs=hbm,
        scratch_shapes=[
            pltpu.VMEM((6, D * H + 64, 128), BF16),
            pltpu.VMEM((H, D, DH), BF16),
            pltpu.VMEM((D, 6 * D), BF16),
            pltpu.VMEM((D, FF), BF16),
            pltpu.VMEM((D, FF), BF16),
            pltpu.VMEM((D, FF), BF16),
            pltpu.VMEM((NBLK, D, TB), BF16),
            pltpu.VMEM((NPAIR * NT, DM, 128), BF16),
            pltpu.VMEM((NPAIR * NT, DM, 128), BF16),
            pltpu.VMEM((25 * 128, 128), F32),
            pltpu.VMEM((NBLK, TB, DP), F32),
            pltpu.VMEM((TB, DP), F32),
            pltpu.VMEM((8, 640, 128), BF16),
            pltpu.VMEM((8, 640, 128), BF16),
            pltpu.VMEM((NBLK, D, TB), F32),
            pltpu.VMEM((NBLK, D, TB), BF16),
            pltpu.VMEM((NBLK, D, TB), BF16),
            pltpu.VMEM((NBLK, TB), F32),
            pltpu.VMEM((3 * H * 2, D, 128), BF16),
            pltpu.VMEM((NPAIR, D, 128), BF16),
            pltpu.VMEM((4, NPAIR * 128, 128), BF16),
            pltpu.VMEM((2, NPAIR, 40, 128), F32),
            pltpu.VMEM((2, 80, 128), BF16),
            pltpu.VMEM((NM, D), BF16),
            pltpu.VMEM((D,), BF16),
            pltpu.VMEM((1, D), BF16),
            pltpu.SMEM((1,), jnp.int32),
            pltpu.SemaphoreType.DMA((24,)),
            pltpu.SemaphoreType.DMA((NBLK,)),
            pltpu.SemaphoreType.DMA((3,)),
            pltpu.SemaphoreType.DMA((NBLK,)),
        ],
        compiler_params=pltpu.CompilerParams(vmem_limit_bytes=110 * 1024 * 1024,
                                             disable_semaphore_checks=True),
    )(xt, mem0, wq, wk, wv, wot, B_w_r, B_w_gate, B_w_up, wdt, c, w_mod)
    return jnp.transpose(out_t).reshape(1, S, D)


def pallas_adaLN_cond__memory_aug_recurrent_mem_tr__moe_arch_mod__prompt_kernel(
    A_x, A_mem0, A_Wq, A_Wk, A_Wv, A_Wo, A_seg_len, B_x, B_w_r, B_w_gate, B_w_up,
    B_w_down, c, w_mod,
):
    del A_seg_len, B_x
    return _run(A_x, A_mem0, A_Wq, A_Wk, A_Wv, A_Wo, B_w_r, B_w_gate, B_w_up, B_w_down,
                c, w_mod)
```
